```python
import os as _os
_os.environ.setdefault("JAX_PLATFORMS", "cpu")
import jax
import jax.numpy as jnp

def _softmax(x, axis=-1):
    return jax.nn.softmax(x, axis=axis)
def _gelu(x):
    return jax.nn.gelu(x, approximate=True)
def _silu(x):
    return jax.nn.silu(x)
def _sigmoid(x):
    return jax.nn.sigmoid(x)
def _layernorm(x, axis=-1, eps=1e-5):
    m = jnp.mean(x, axis=axis, keepdims=True)
    v = jnp.var(x, axis=axis, keepdims=True)
    return (x - m) / jnp.sqrt(v + eps)
def _scatter_add(tgt, idx, src, axis=0):
    return tgt.at[idx].add(src)
def _segment_sum(src, seg, n):
    return jax.ops.segment_sum(src, seg, n)
class _Rng:
    def __init__(self, key):
        self._k = key
    def _next(self):
        self._k, sub = jax.random.split(self._k)
        return sub
    def normal(self, shape):
        return jax.random.normal(self._next(), shape, dtype=jnp.bfloat16)
    def randint(self, lo, hi, shape):
        return jax.random.randint(self._next(), shape, lo, hi, dtype=jnp.int32)
    def uniform(self, shape, lo=0.0, hi=1.0):
        return jax.random.uniform(self._next(), shape, jnp.bfloat16, lo, hi)
    def permutation(self, n):
        return jax.random.permutation(self._next(), n)


kernel_name = 'standalone__linear_kernel_hedgehog__prompt'

def setup_inputs():
    _rng = _Rng(jax.random.key(int.from_bytes(__import__("os").urandom(4), "little")))
    _w = (lambda a: (lambda t: t.astype(jnp.bfloat16) if jnp.issubdtype(t.dtype, jnp.floating) else t)(jnp.asarray(a)))
    B, S, D, H = 1, 2048, 1024, 32
    Dh = D // H
    return {
        "x": _w((lambda *s: _rng.normal(s) * 0.4)(B, S, D)),
        "wqkv": _w((lambda *s: _rng.normal(s) * 0.4)(D, 3 * D)),
        "w_phi": _w((lambda *s: _rng.normal(s) * 0.4)(H, Dh, Dh) * (Dh ** -0.5)),
        "wo": _w((lambda *s: _rng.normal(s) * 0.05)(D, D)),
    }

def reference(x, wqkv, w_phi, wo):
    B, S, D = x.shape
    H = 32; Dh = D // H
    qkv = (lambda x, *d: x.transpose(*d))((x @ wqkv).reshape(B, S, 3, H, Dh), 2, 0, 3, 1, 4)
    q, k, v = qkv[0], qkv[1], qkv[2]
    pq = jnp.einsum("bhsd,hdf->bhsf", q, w_phi)
    pk = jnp.einsum("bhsd,hdf->bhsf", k, w_phi)
    phi_q = jnp.concatenate([_softmax(pq, axis=-1), _softmax(-pq, axis=-1)], axis=-1)
    phi_k = jnp.concatenate([_softmax(pk, axis=-1), _softmax(-pk, axis=-1)], axis=-1)
    kv = jnp.einsum("bhsf,bhsd->bhfd", phi_k, v)
    z  = jnp.einsum("bhsf->bhf", phi_k)
    num = jnp.einsum("bhqf,bhfd->bhqd", phi_q, kv)
    den = jnp.einsum("bhqf,bhf->bhq", phi_q, z)[..., None] + 1e-6
    o = num / den
    return (lambda x, *d: x.transpose(*d))(o, 0, 2, 1, 3).reshape(B, S, D) @ wo
```

```python
import contextlib
import numpy as np
import jax
import jax.numpy as jnp
from jax import lax
from jax.experimental import pallas as pl
from jax.experimental.pallas import tpu as pltpu

S, D, H, DH = 2048, 1024, 32, 32
LOG2E = 1.4426950408889634
NT = (((1,), (1,)), ((), ()))
NN = (((1,), (0,)), ((), ()))
TN = (((0,), (0,)), ((), ()))
f32, bf16 = jnp.float32, jnp.bfloat16
TS = 256
T = S // TS


RCP = [False]
def recip(x):
    if RCP[0]:
        r = pl.reciprocal(x, approx=True)
        return r * (2.0 - x * r)
    return 1.0 / x


def feat(p):
    mx = jnp.max(p, axis=0, keepdims=True)
    mn = jnp.min(p, axis=0, keepdims=True)
    ep = jnp.exp2(p - mx)
    en = jnp.exp2(mn - p)
    sp = jnp.sum(ep, axis=0, keepdims=True)
    sn = jnp.sum(en, axis=0, keepdims=True)
    return ep * recip(sp), en * recip(sn)


def pair_feat(p2):
    a, b = feat(p2[0:32])
    c, d = feat(p2[32:64])
    return jnp.concatenate([a, b, c, d], axis=0)


def make(scopes=False, U2=2, iss=('p1', 'k2', 'k3', 'k4', 'k6', 'v7', 'x1', 'q1', None), RC=64, o1='A', o2='A', fqpos=3, stage=False, flags=None, rcp=False, xu=False, hyb=False):
    RCP[0] = rcp
    def scope(n):
        return jax.named_scope(n) if scopes else contextlib.nullcontext()

    def kernel(x_hbm, wqkv_hbm, wphi_hbm, wo_hbm, out_hbm,
               x_v, wq_v, wk_v, wv_v, wphi_v, wo_v, wkT, wqT, wvT, bd_v, kv_acc, kvb, zacc, car0, car7, cph7, carv, caro, acc, out_v, phb, xu_v,
               sem):
        def cp_phi(a, b, s): return pltpu.make_async_copy(wphi_hbm.at[pl.ds(a * 128, (b - a) * 128), :], wphi_v.at[pl.ds(a * 128, (b - a) * 128), :], sem.at[s])
        def cp_q(G, s): return pltpu.make_async_copy(wqkv_hbm.at[:, pl.ds(G * 128, 128)], wq_v.at[G], sem.at[s])
        def cp_k(G, s): return pltpu.make_async_copy(wqkv_hbm.at[:, pl.ds(D + G * 128, 128)], wk_v.at[G], sem.at[s])
        def cp_v(G, s): return pltpu.make_async_copy(wqkv_hbm.at[:, pl.ds(2 * D + G * 128, 128)], wv_v.at[G], sem.at[s])
        def cp_x(t, s): return pltpu.make_async_copy(x_hbm.at[pl.ds((t % T) * TS, TS), :], x_v.at[t], sem.at[s])
        def cp_xd(t, s):
            r0 = pl.multiple_of(jnp.where(t >= T, 0, t) * TS, TS)
            return pltpu.make_async_copy(x_hbm.at[pl.ds(r0, TS), :], x_v.at[t], sem.at[s])
        def cp_qd(G, s): return pltpu.make_async_copy(wqkv_hbm.at[:, pl.ds(pl.multiple_of(G * 128, 128), 128)], wq_v.at[G], sem.at[s])
        cp_wo = pltpu.make_async_copy(wo_hbm, wo_v, sem.at[7])

        groups = [['p0', 'k0'], ['x0', 'k1'], ['p1', 'v0', 'k2'], ['p2', 'v1', 'k3'], ['v2', 'k4'], ['v3', 'k5', 'v4', 'k6'], ['v5', 'k7', 'v6', 'v7'], ['x1', 'q0']]
        D_ = {}
        for s, grp in enumerate(groups):
            for n in grp:
                kind, i = n[0], int(n[1:])
                if kind == 'p':
                    a, b = [(0, 2), (2, 4), (4, 8)][i]
                    D_[n] = lambda a=a, b=b, s=s: cp_phi(a, b, s)
                else:
                    D_[n] = lambda kind=kind, i=i, s=s: dict(q=cp_q, k=cp_k, v=cp_v, x=cp_x)[kind](i, s)
        order = sum(groups, [])
        for i in range(7):
            D_[f"x{i+2}"] = lambda i=i: cp_x(i + 2, i)
            D_[f"q{i+1}"] = lambda i=i: cp_q(i + 1, i)
            order += [f"x{i+2}", f"q{i+1}"]
        D_["o"] = lambda: cp_wo
        order += ["o"]
        pos = [0]
        def issue_to(name):
            i = len(order) - 1 if name is None else order.index(name)
            while pos[0] <= i:
                D_[order[pos[0]]]().start(); pos[0] += 1
        def wait(k):
            for n in groups[k]:
                assert order.index(n) < pos[0], n
                D_[n]().wait()

        rowh = lax.broadcasted_iota(jnp.int32, (32, 128), 1) // 32

        def BD(G):
            Tm = wphi_v[G * 128:(G + 1) * 128, :].astype(f32).T
            bd_v[G] = jnp.concatenate([jnp.where(rowh == j, Tm, 0.0) for j in range(4)], axis=0).astype(bf16)

        def fold(G, w_ref):
            return (lax.dot_general(bd_v[G], w_ref[G], NT, preferred_element_type=f32) * LOG2E).astype(bf16)

        def Fk(G):
            wkT[G] = fold(G, wk_v)

        def Tv(G):
            wvT[G] = wv_v[G].T

        def xconv(t):
            if xu:
                xu_v[t] = pltpu.bitcast(x_v[t], jnp.uint32)

        def proj(w_ref, wi, t):
            xx = pltpu.bitcast(xu_v[t], bf16) if xu else x_v[t]
            return lax.dot_general(w_ref[wi], xx, NT, preferred_element_type=f32)

        def projv(G, t):
            return proj(wvT, G, t).astype(bf16)

        def SMk(p, G):
            out = []
            for j in range(2):
                ph = pair_feat(p[64 * j:64 * j + 64])
                zacc[2 * G + j] += ph[:, 0:128] + ph[:, 128:256]
                out.append(ph.astype(bf16))
            return tuple(out)

        def den_r(ph, g):
            zb = zacc[g]
            rs = []
            for hh in range(2):
                cols = []
                for l in range(TS // 128):
                    pr = ph[64 * hh:64 * hh + 64, 128 * l:128 * l + 128] * zb[64 * hh:64 * hh + 64]
                    cols.append(jnp.sum(pr, axis=0, keepdims=True))
                rs.append(recip(jnp.concatenate(cols, axis=1) + 1e-6))
            return rs

        def SMq(p, G):
            out = []; rr = []
            for j in range(2):
                ph = pair_feat(p[64 * j:64 * j + 64])
                rr.append(den_r(ph, 2 * G + j))
                out.append(ph.astype(bf16))
            return tuple(out), tuple(rr)

        def stg(phi, G):
            if not stage:
                return phi
            phb[G, 0] = phi[0]
            phb[G, 1] = phi[1]
            return (phb[G, 0], phb[G, 1])

        def KV(phi, v, G, first):
            for j in range(2):
                g = 2 * G + j
                d = lax.dot_general(v[64 * j:64 * j + 64], phi[j], NT, preferred_element_type=f32)
                if not first:
                    d = d + kv_acc[g]
                kv_acc[g] = d

        pk = {}; ph = {}; pv = {}
        issue_to(iss[0])
        zacc[...] = jnp.zeros(zacc.shape, f32)
        kv_acc[14] = jnp.zeros((64, 128), f32)
        kv_acc[15] = jnp.zeros((64, 128), f32)
        with scope("w0"):
            wait(0); issue_to(iss[1])
        with scope("a0"):
            BD(0); Fk(0); BD(1)
        with scope("w1"):
            wait(1); issue_to(iss[2])
        with scope("a1"):
            xconv(0)
            pk[0] = proj(wkT, 0, 0); Fk(1)
        with scope("w2"):
            wait(2); issue_to(iss[3])
        with scope("a2"):
            BD(2); Tv(0); BD(3)
            pk[1] = proj(wkT, 1, 0)
            ph[0] = SMk(pk.pop(0), 0)
            Fk(2)
            pv[0] = projv(0, 0)
        with scope("w3"):
            wait(3); issue_to(iss[4])
        with scope("a3"):
            Tv(1)
            pk[2] = proj(wkT, 2, 0)
            ph[1] = SMk(pk.pop(1), 1)
            for G in range(4, 8): BD(G)
            Fk(3)
            KV(ph.pop(0), pv.pop(0), 0, True)
            pv[1] = projv(1, 0)
        with scope("w4"):
            wait(4); issue_to(iss[5])
        with scope("a4"):
            Tv(2)
            pk[3] = proj(wkT, 3, 0)
            ph[2] = SMk(pk.pop(2), 2)
            Fk(4)
            KV(ph.pop(1), pv.pop(1), 1, True)
            pv[2] = projv(2, 0)
        with scope("w5"):
            wait(5); issue_to(iss[6])
        with scope("a5"):
            Tv(3); Tv(4)
            pk[4] = proj(wkT, 4, 0)
            ph[3] = SMk(pk.pop(3), 3)
            Fk(5)
            KV(ph.pop(2), pv.pop(2), 2, True)
            pv[3] = projv(3, 0)
            pk[5] = proj(wkT, 5, 0)
            ph[4] = SMk(pk.pop(4), 4)
            Fk(6)
            KV(ph.pop(3), pv.pop(3), 3, True)
            pv[4] = projv(4, 0)
        with scope("w6"):
            wait(6); issue_to(iss[7])
        with scope("a6"):
            Tv(5); Tv(6); Tv(7)
            pk[6] = proj(wkT, 6, 0)
            ph[5] = SMk(pk.pop(5), 5)
            Fk(7)
            KV(ph.pop(4), pv.pop(4), 4, True)
            pv[5] = projv(5, 0)
            car7[...] = proj(wkT, 7, 0)
            ph[6] = SMk(pk.pop(6), 6)
            KV(ph.pop(5), pv.pop(5), 5, True)
            pv[6] = projv(6, 0)
        with scope("w7"):
            wait(7); issue_to(iss[8])
        with scope("a7"):
            xconv(1)
            car0[...] = proj(wkT, 0, 1)
            if hyb:
                q7 = SMk(car7[...], 7)
                cph7[0] = q7[0]; cph7[1] = q7[1]
            wkT[8] = fold(0, wq_v)
            carv[...] = projv(7, 0)
            KV(ph.pop(6), pv.pop(6), 6, True)

        def p1(i, carry):
            t = 1 + i
            cp_xd(t + 1, i).wait()
            cp_qd(i + 1, i).wait()
            xconv(t + 1)
            ph = {-1: (cph7[0], cph7[1]) if hyb else stg(SMk(car7[...], 7), 7)}
            pv = {-1: carv[...]}
            pk = car0[...]
            for G in range(8):
                def do_K():
                    if G < 7:
                        return proj(wkT, G + 1, t)
                    car0[...] = proj(wkT, jnp.where(t + 1 >= T, 8, 0), t + 1)
                def do_V():
                    if G < 7:
                        pv[G] = projv(G, t)
                    else:
                        carv[...] = projv(G, t)
                def do_KV():
                    KV(ph.pop(G - 1), pv.pop(G - 1), 7 if G == 0 else G - 1, False)
                def do_SM():
                    if G < 7:
                        ph[G] = stg(SMk(pk, G), G)
                    elif hyb:
                        q7 = SMk(pk, 7)
                        cph7[0] = q7[0]; cph7[1] = q7[1]
                    else:
                        car7[...] = pk
                if o1 == 'A':
                    npk = do_K(); do_V(); do_KV(); do_SM()
                elif o1 == 'B':
                    npk = do_K(); do_SM(); do_V(); do_KV()
                elif o1 == 'C':
                    do_SM(); npk = do_K(); do_V(); do_KV()
                elif o1 == 'D':
                    npk = do_K(); do_V(); do_SM(); do_KV()
                elif o1 == 'E':
                    do_V(); npk = do_K(); do_SM(); do_KV()
                elif o1 == 'F':
                    do_V(); do_SM(); npk = do_K(); do_KV()
                pk = npk
                if G == fqpos:
                    wqT[i + 1] = fold(i + 1, wq_v)
            return carry

        with scope("b_p1"):
            lax.fori_loop(0, T - 1, p1, 0)

        def N2(phi, rr, G):
            os_ = []
            for j in range(2):
                nd = lax.dot_general(kvb[2 * G + j], phi[j], NN, preferred_element_type=f32)
                os_ += [nd[0:32] * rr[j][0], nd[32:64] * rr[j][1]]
            return jnp.concatenate(os_, axis=0).astype(bf16)

        def cp_out(t):
            return pltpu.make_async_copy(out_v.at[t], out_hbm.at[pl.ds(t * TS, TS), :], sem.at[0])

        def cp_out_c(t, m, n):
            return pltpu.make_async_copy(out_v.at[t, pl.ds(m * RC, RC), pl.ds(n * 512, 512)], out_hbm.at[pl.ds(t * TS + m * RC, RC), pl.ds(n * 512, 512)], sem.at[0])

        def OP(oT, t, G):
            res = lax.dot_general(oT, wo_v[G * 128:(G + 1) * 128, :], TN, preferred_element_type=f32)
            if G == 0:
                acc[...] = res
            elif G < 7:
                acc[...] += res
            else:
                out_v[t] = (acc[...] + res).astype(bf16)
                cp_out(t).start()

        def Q(G, t):
            return proj(wkT, 8, t) if G == 0 else proj(wqT, G, t)

        with scope("c_p2t0"):
            r = lax.broadcasted_iota(jnp.int32, (64, 128), 0)
            c = lax.broadcasted_iota(jnp.int32, (64, 128), 1)
            mask = (r // 32) == (c // 64)
            cp_wo.wait()
            for g in range(14):
                zacc[g] = jnp.broadcast_to(jnp.sum(zacc[g], axis=1, keepdims=True), (128, 128))
            for g in range(14):
                kvb[g] = jnp.where(mask, kv_acc[g], 0.0).astype(bf16)
            npq = Q(1, 0)
            phi, rr = SMq(car0[...], 0)
            ph7 = (cph7[0], cph7[1]) if hyb else SMk(car7[...], 7)
            oT = None
            for G in range(8):
                pq = npq
                if G == 1:
                    for j in range(2):
                        d = lax.dot_general(carv[64 * j:64 * j + 64], ph7[j], NT, preferred_element_type=f32) + kv_acc[14 + j]
                        kvb[14 + j] = jnp.where(mask, d, 0.0).astype(bf16)
                        zacc[14 + j] = jnp.broadcast_to(jnp.sum(zacc[14 + j], axis=1, keepdims=True), (128, 128))
                if G < 6:
                    npq = Q(G + 2, 0)
                elif G == 6:
                    car0[...] = Q(0, 1)
                noT = N2(phi, rr, G)
                if G < 7:
                    phi, rr = SMq(pq, G + 1)
                else:
                    caro[...] = noT
                if G > 0:
                    OP(oT, 0, G - 1)
                oT = noT

        def p2_tile(t, pq0, oT, lastt, final=False):
            npq = Q(1, t)
            phi, rr = SMq(pq0, 0)
            OP(oT, t - 1, 7)
            oT = N2(phi, rr, 0)
            phi, rr = SMq(npq, 1)
            nq0 = None
            for G in range(1, 8):
                if G < 7:
                    pq = Q(G + 1, t)
                elif not final:
                    nq0 = Q(0, t + 1)
                    if lastt:
                        car0[...] = nq0
                noT = N2(phi, rr, G)
                if G < 7:
                    phi, rr = SMq(pq, G + 1)
                elif lastt and not final:
                    caro[...] = noT
                OP(oT, t, G - 1)
                oT = noT
            return nq0, oT

        def p2(i, carry):
            t = 1 + U2 * i
            pq0 = car0[...]
            oT = caro[...]
            for u in range(U2):
                pq0, oT = p2_tile(t + u, pq0, oT, u == U2 - 1)
            return carry

        with scope("d_p2"):
            lax.fori_loop(0, 6 // U2, p2, 0)

        with scope("e_epi"):
            t = T - 1
            _, oT = p2_tile(t, car0[...], caro[...], True, True)
            o = oT.T
            for n in range(2):
                for m in range(TS // RC):
                    res = jnp.dot(o[m * RC:(m + 1) * RC], wo_v[7 * 128:8 * 128, n * 512:(n + 1) * 512], preferred_element_type=f32)
                    out_v[t, m * RC:(m + 1) * RC, n * 512:(n + 1) * 512] = (acc[m * RC:(m + 1) * RC, n * 512:(n + 1) * 512] + res).astype(bf16)
                    cp_out_c(t, m, n).start()
        with scope("f_tail"):
            for tt in range(T - 1):
                cp_out(tt).wait()
            for n in range(2):
                for m in range(TS // RC):
                    cp_out_c(t, m, n).wait()

    def run(x, wqkv, w_phi, wo):
        any_spec = pl.BlockSpec(memory_space=pl.ANY)
        out = pl.pallas_call(
            kernel,
            out_shape=jax.ShapeDtypeStruct((S, D), bf16),
            in_specs=[any_spec] * 4,
            out_specs=any_spec,
            scratch_shapes=[
                pltpu.VMEM((T + 1, TS, D), bf16),
                pltpu.VMEM((8, D, 128), bf16),
                pltpu.VMEM((8, D, 128), bf16),
                pltpu.VMEM((8, D, 128), bf16),
                pltpu.VMEM((H * DH, DH), bf16),
                pltpu.VMEM((D, D), bf16),
                pltpu.VMEM((9, 128, D), bf16),
                pltpu.VMEM((8, 128, D), bf16),
                pltpu.VMEM((8, 128, D), bf16),
                pltpu.VMEM((8, 128, 128), bf16),
                pltpu.VMEM((16, 64, 128), f32),
                pltpu.VMEM((16, 64, 128), bf16),
                pltpu.VMEM((16, 128, 128), f32),
                pltpu.VMEM((128, TS), f32),
                pltpu.VMEM((128, TS), f32),
                pltpu.VMEM((2, 128, TS), bf16),
                pltpu.VMEM((128, TS), bf16),
                pltpu.VMEM((128, TS), bf16),
                pltpu.VMEM((TS, D), f32),
                pltpu.VMEM((T, TS, D), bf16),
                pltpu.VMEM((9, 2, 128, TS), bf16),
                pltpu.VMEM((T + 1, TS // 2, D), jnp.uint32),
                pltpu.SemaphoreType.DMA((8,)),
            ],
            compiler_params=pltpu.CompilerParams(vmem_limit_bytes=100 * 1024 * 1024, flags=flags),
            name="hh8",
        )(x.reshape(S, D), wqkv, w_phi.reshape(H * DH, DH), wo)
        return out.reshape(1, S, D)

    return jax.jit(run)


_impl = make(U2=2, rcp=True, xu=True, hyb=True)


@jax.jit
def pallas_standalone__linear_kernel_hedgehog__prompt_kernel(x, wqkv, w_phi, wo):
    return _impl(x, wqkv, w_phi, wo)
```

```python
import jax
import jax.numpy as jnp
from jax import lax
import jax.experimental.pallas as pl
import jax.experimental.pallas.tpu as pltpu

S, D, H, DH = 2048, 1024, 32, 32
TS = 256
T = S // TS
U2 = 3
RC = 64
LOG2E = 1.4426950408889634
NT = (((1,), (1,)), ((), ()))
NN = (((1,), (0,)), ((), ()))
TN = (((0,), (0,)), ((), ()))
f32, bf16 = jnp.float32, jnp.bfloat16


def _recip(x):
    r = pl.reciprocal(x, approx=True)
    return r * (2.0 - x * r)


def _allred(x, op):
    y = x[0:8]
    for i in range(1, x.shape[0] // 8):
        y = op(y, x[8 * i:8 * i + 8])
    y = op(y, pltpu.roll(y, 4, 0))
    return op(y, pltpu.roll(y, 2, 0))


def _pair_feat(p2):
    n = p2.shape[1]
    mx = _allred(p2, jnp.maximum)
    mn = _allred(p2, jnp.minimum)
    p3 = p2.reshape(8, 8, n)
    ep = jnp.exp2(p3 - mx[None]).reshape(64, n)
    en = jnp.exp2(mn[None] - p3).reshape(64, n)
    rp = _recip(_allred(ep, jnp.add))
    rn = _recip(_allred(en, jnp.add))
    a = (ep.reshape(8, 8, n) * rp[None]).reshape(64, n)
    b = (en.reshape(8, 8, n) * rn[None]).reshape(64, n)
    return jnp.concatenate([a, b], axis=0)


def _kernel(x_hbm, wqkv_hbm, wphi_hbm, wo_hbm, out_hbm,
            x_v, wq_v, wk_v, wv_v, wphi_v, wo_v, wkT, wqT, wvT, bd_v, kv_acc, kvb, zacc,
            car0, car7, cph7, carv, caro, acc, out_v, bdtmp, xu_v, sem):
    def cp_phi(a, b, s):
        rows = pl.ds(a * 128, (b - a) * 128)
        return pltpu.make_async_copy(wphi_hbm.at[rows, :], wphi_v.at[rows, :], sem.at[s])

    def cp_q(G, s):
        return pltpu.make_async_copy(wqkv_hbm.at[:, pl.ds(G * 128, 128)], wq_v.at[G], sem.at[s])

    def cp_k(G, s):
        return pltpu.make_async_copy(wqkv_hbm.at[:, pl.ds(D + G * 128, 128)], wk_v.at[G], sem.at[s])

    def cp_v(G, s):
        return pltpu.make_async_copy(wqkv_hbm.at[:, pl.ds(2 * D + G * 128, 128)], wv_v.at[G], sem.at[s])

    def cp_x(t, s):
        return pltpu.make_async_copy(x_hbm.at[pl.ds((t % T) * TS, TS), :], x_v.at[t], sem.at[s])

    def cp_x_dyn(t, s):
        r0 = pl.multiple_of(jnp.where(t >= T, 0, t) * TS, TS)
        return pltpu.make_async_copy(x_hbm.at[pl.ds(r0, TS), :], x_v.at[t], sem.at[s])

    def cp_q_dyn(G, s):
        cols = pl.ds(pl.multiple_of(G * 128, 128), 128)
        return pltpu.make_async_copy(wqkv_hbm.at[:, cols], wq_v.at[G], sem.at[s])

    cp_wo = pltpu.make_async_copy(wo_hbm, wo_v, sem.at[7])

    groups = [['p0', 'k0'], ['x0', 'k1'], ['p1', 'v0', 'k2'], ['p2', 'v1', 'k3'],
              ['v2', 'k4', 'v3', 'k5'], ['v4', 'k6', 'v5', 'k7', 'v6'], ['v7', 'x1', 'q0']]
    dmas = {}
    for s, grp in enumerate(groups):
        for n in grp:
            kind, i = n[0], int(n[1:])
            if kind == 'p':
                a, b = [(0, 2), (2, 4), (4, 8)][i]
                dmas[n] = lambda a=a, b=b, s=s: cp_phi(a, b, s)
            else:
                fn = {'q': cp_q, 'k': cp_k, 'v': cp_v, 'x': cp_x}[kind]
                dmas[n] = lambda fn=fn, i=i, s=s: fn(i, s)
    order = [n for grp in groups for n in grp]
    for i in range(7):
        dmas[f"x{i + 2}"] = lambda i=i: cp_x(i + 2, i)
        dmas[f"q{i + 1}"] = lambda i=i: cp_q(i + 1, i)
        order += [f"x{i + 2}", f"q{i + 1}"]
    dmas["o"] = lambda: cp_wo
    order += ["o"]
    pos = [0]

    def issue_to(name):
        last = len(order) - 1 if name is None else order.index(name)
        while pos[0] <= last:
            dmas[order[pos[0]]]().start()
            pos[0] += 1

    def wait(k):
        for n in groups[k]:
            assert order.index(n) < pos[0], n
            dmas[n]().wait()

    lane_head = lax.broadcasted_iota(jnp.int32, (32, 128), 1) // 32

    def BD(G):
        tm = wphi_v[G * 128:(G + 1) * 128, :].astype(f32).T
        for hh in range(4):
            rows = pl.ds(64 * (hh // 2) + hh % 2, 32, stride=2)
            bdtmp[G, rows, :] = jnp.where(lane_head == hh, tm, 0.0)
        bd_v[G] = bdtmp[G].astype(bf16)

    def fold(G, w_ref):
        w = lax.dot_general(bd_v[G], w_ref[G], NT, preferred_element_type=f32)
        return (w * LOG2E).astype(bf16)

    def Fk(G):
        wkT[G] = fold(G, wk_v)

    def Tv(G):
        wvT[G] = wv_v[G].T

    def xconv(t):
        xu_v[t] = pltpu.bitcast(x_v[t], jnp.uint32)

    def proj(w_ref, wi, t):
        return lax.dot_general(w_ref[wi], pltpu.bitcast(xu_v[t], bf16), NT, preferred_element_type=f32)

    def projv(G, t):
        return proj(wvT, G, t).astype(bf16)

    def SMk(p, G):
        out = []
        for j in range(2):
            ph = _pair_feat(p[64 * j:64 * j + 64])
            zacc[2 * G + j] += ph[:, 0:128] + ph[:, 128:256]
            out.append(ph.astype(bf16))
        return tuple(out)

    def den_r(ph, g):
        zb = zacc[g]
        cols = [_allred(ph[:, 128 * l:128 * l + 128] * zb, jnp.add) for l in range(TS // 128)]
        r = _recip(jnp.concatenate(cols, axis=1) + 1e-6)
        rs = pltpu.roll(r, 1, 0)
        even = (lax.broadcasted_iota(jnp.int32, (8, TS), 0) % 2) == 0
        return [jnp.where(even, r, rs), jnp.where(even, rs, r)]

    def SMq(p, G):
        out, rr = [], []
        for j in range(2):
            ph = _pair_feat(p[64 * j:64 * j + 64])
            rr.append(den_r(ph, 2 * G + j))
            out.append(ph.astype(bf16))
        return tuple(out), tuple(rr)

    def KV(phi, v, G, first):
        for j in range(2):
            g = 2 * G + j
            d = lax.dot_general(v[64 * j:64 * j + 64], phi[j], NT, preferred_element_type=f32)
            if not first:
                d = d + kv_acc[g]
            kv_acc[g] = d

    pk, ph, pv = {}, {}, {}
    issue_to('p1')
    zacc[...] = jnp.zeros(zacc.shape, f32)
    kv_acc[14] = jnp.zeros((64, 128), f32)
    kv_acc[15] = jnp.zeros((64, 128), f32)

    wait(0); issue_to('k2')
    BD(0); Fk(0); BD(1)

    wait(1); issue_to('k3')
    xconv(0)
    pk[0] = proj(wkT, 0, 0); Fk(1)

    wait(2); issue_to('k5')
    BD(2); Tv(0); BD(3)
    pk[1] = proj(wkT, 1, 0)
    ph[0] = SMk(pk.pop(0), 0)
    Fk(2)
    pv[0] = projv(0, 0)

    wait(3); issue_to('v6')
    Tv(1)
    pk[2] = proj(wkT, 2, 0)
    ph[1] = SMk(pk.pop(1), 1)
    for G in range(4, 8):
        BD(G)
    Fk(3)
    KV(ph.pop(0), pv.pop(0), 0, True)
    pv[1] = projv(1, 0)

    wait(4); issue_to('q0')
    Tv(2); Tv(3)
    pk[3] = proj(wkT, 3, 0)
    ph[2] = SMk(pk.pop(2), 2)
    Fk(4)
    KV(ph.pop(1), pv.pop(1), 1, True)
    pv[2] = projv(2, 0)
    pk[4] = proj(wkT, 4, 0)
    ph[3] = SMk(pk.pop(3), 3)
    Fk(5)
    KV(ph.pop(2), pv.pop(2), 2, True)
    pv[3] = projv(3, 0)

    wait(5); issue_to('q1')
    Tv(4); Tv(5); Tv(6)
    pk[5] = proj(wkT, 5, 0)
    ph[4] = SMk(pk.pop(4), 4)
    Fk(6)
    Fk(7)
    KV(ph.pop(3), pv.pop(3), 3, True)
    pv[4] = projv(4, 0)
    pk[6] = proj(wkT, 6, 0)
    ph[5] = SMk(pk.pop(5), 5)
    pv[5] = projv(5, 0)
    KV(ph.pop(4), pv.pop(4), 4, True)
    car7[...] = proj(wkT, 7, 0)
    ph[6] = SMk(pk.pop(6), 6)
    pv[6] = projv(6, 0)
    KV(ph.pop(5), pv.pop(5), 5, True)

    wait(6); issue_to(None)
    Tv(7)
    xconv(1)
    car0[...] = proj(wkT, 0, 1)
    q7 = SMk(car7[...], 7)
    cph7[0] = q7[0]
    cph7[1] = q7[1]
    wkT[8] = fold(0, wq_v)
    KV(ph.pop(6), pv.pop(6), 6, True)
    carv[...] = projv(7, 0)

    def phase1(i, carry):
        t = 1 + i
        cp_x_dyn(t + 1, i).wait()
        cp_q_dyn(t, i).wait()
        pk_ = car0[...]
        ph_ = {-1: (cph7[0], cph7[1])}
        pv_ = {-1: carv[...]}
        xconv(t + 1)
        for G in range(8):
            if G < 7:
                npk = proj(wkT, G + 1, t)
            else:
                npk = proj(wkT, jnp.where(t + 1 >= T, 8, 0), t + 1)
                car0[...] = npk
            pv_[G] = projv(G, t)
            if G == 7:
                carv[...] = pv_[G]
            KV(ph_.pop(G - 1), pv_.pop(G - 1), 7 if G == 0 else G - 1, False)
            ph_[G] = SMk(pk_, G)
            if G == 7:
                cph7[0] = ph_[G][0]
                cph7[1] = ph_[G][1]
            pk_ = npk
            if G == 3:
                wqT[i + 1] = fold(i + 1, wq_v)
        return carry

    lax.fori_loop(0, T - 1, phase1, 0)

    def N2(phi, rr, G):
        os_ = []
        for j in range(2):
            nd = lax.dot_general(kvb[2 * G + j], phi[j], NN, preferred_element_type=f32)
            os_ += [(nd[32 * e:32 * e + 32].reshape(4, 8, TS) * rr[j][e][None]).reshape(32, TS)
                    for e in range(2)]
        return jnp.concatenate(os_, axis=0).astype(bf16)

    def cp_out(t):
        return pltpu.make_async_copy(out_v.at[t], out_hbm.at[pl.ds(t * TS, TS), :], sem.at[0])

    def cp_out_chunk(t, m, n):
        return pltpu.make_async_copy(
            out_v.at[t, pl.ds(m * RC, RC), pl.ds(n * 512, 512)],
            out_hbm.at[pl.ds(t * TS + m * RC, RC), pl.ds(n * 512, 512)], sem.at[0])

    def OP(oT, t, G):
        res = lax.dot_general(oT, wo_v[G * 128:(G + 1) * 128, :], TN, preferred_element_type=f32)
        if G == 0:
            acc[...] = res
        elif G < 7:
            acc[...] += res
        else:
            out_v[t] = (acc[...] + res).astype(bf16)
            cp_out(t).start()

    def Q(G, t):
        return proj(wkT, 8, t) if G == 0 else proj(wqT, G, t)

    r = lax.broadcasted_iota(jnp.int32, (64, 128), 0)
    c = lax.broadcasted_iota(jnp.int32, (64, 128), 1)
    mask = (r // 32) == (c % 2)
    cp_wo.wait()
    for g in range(14):
        zacc[g] = jnp.broadcast_to(jnp.sum(zacc[g], axis=1, keepdims=True), (128, 128))
    for g in range(14):
        kvb[g] = jnp.where(mask, kv_acc[g], 0.0).astype(bf16)
    npq = Q(1, 0)
    phi, rr = SMq(car0[...], 0)
    ph7 = (cph7[0], cph7[1])
    oT = None
    for G in range(8):
        pq = npq
        if G == 1:
            for j in range(2):
                d = lax.dot_general(carv[64 * j:64 * j + 64], ph7[j], NT,
                                    preferred_element_type=f32) + kv_acc[14 + j]
                kvb[14 + j] = jnp.where(mask, d, 0.0).astype(bf16)
                zacc[14 + j] = jnp.broadcast_to(
                    jnp.sum(zacc[14 + j], axis=1, keepdims=True), (128, 128))
        if G < 6:
            npq = Q(G + 2, 0)
        elif G == 6:
            car0[...] = Q(0, 1)
        noT = N2(phi, rr, G)
        if G < 7:
            phi, rr = SMq(pq, G + 1)
        else:
            caro[...] = noT
        if G > 0:
            OP(oT, 0, G - 1)
        oT = noT

    def p2_tile(t, pq0, oT, store, final=False):
        npq = Q(1, t)
        phi, rr = SMq(pq0, 0)
        OP(oT, t - 1, 7)
        oT = N2(phi, rr, 0)
        phi, rr = SMq(npq, 1)
        nq0 = None
        for G in range(1, 8):
            if G < 7:
                pq = Q(G + 1, t)
            elif not final:
                nq0 = Q(0, t + 1)
                if store:
                    car0[...] = nq0
            noT = N2(phi, rr, G)
            if G < 7:
                phi, rr = SMq(pq, G + 1)
            elif store:
                caro[...] = noT
            OP(oT, t, G - 1)
            oT = noT
        return nq0, oT

    def phase2(i, carry):
        t = 1 + U2 * i
        pq0 = car0[...]
        oT = caro[...]
        for u in range(U2):
            pq0, oT = p2_tile(t + u, pq0, oT, u == U2 - 1)
        return carry

    lax.fori_loop(0, (T - 2) // U2, phase2, 0)

    t = T - 1
    _, oT = p2_tile(t, car0[...], caro[...], False, True)
    o = oT.T
    for n in range(2):
        for m in range(TS // RC):
            rows, cols = slice(m * RC, (m + 1) * RC), slice(n * 512, (n + 1) * 512)
            res = jnp.dot(o[rows], wo_v[7 * 128:8 * 128, cols], preferred_element_type=f32)
            out_v[t, rows, cols] = (acc[rows, cols] + res).astype(bf16)
            cp_out_chunk(t, m, n).start()
    for tt in range(T - 1):
        cp_out(tt).wait()
    for n in range(2):
        for m in range(TS // RC):
            cp_out_chunk(t, m, n).wait()


def _run(x, wqkv, w_phi, wo, interpret=False):
    any_spec = pl.BlockSpec(memory_space=pl.ANY)
    out = pl.pallas_call(
        _kernel,
        out_shape=jax.ShapeDtypeStruct((S, D), bf16),
        in_specs=[any_spec] * 4,
        out_specs=any_spec,
        scratch_shapes=[
            pltpu.VMEM((T + 1, TS, D), bf16),
            pltpu.VMEM((8, D, 128), bf16),
            pltpu.VMEM((8, D, 128), bf16),
            pltpu.VMEM((8, D, 128), bf16),
            pltpu.VMEM((H * DH, DH), bf16),
            pltpu.VMEM((D, D), bf16),
            pltpu.VMEM((9, 128, D), bf16),
            pltpu.VMEM((8, 128, D), bf16),
            pltpu.VMEM((8, 128, D), bf16),
            pltpu.VMEM((8, 128, 128), bf16),
            pltpu.VMEM((16, 64, 128), f32),
            pltpu.VMEM((16, 64, 128), bf16),
            pltpu.VMEM((16, 128, 128), f32),
            pltpu.VMEM((128, TS), f32),
            pltpu.VMEM((128, TS), f32),
            pltpu.VMEM((2, 128, TS), bf16),
            pltpu.VMEM((128, TS), bf16),
            pltpu.VMEM((128, TS), bf16),
            pltpu.VMEM((TS, D), f32),
            pltpu.VMEM((T, TS, D), bf16),
            pltpu.VMEM((8, 128, 128), f32),
            pltpu.VMEM((T + 1, TS // 2, D), jnp.uint32),
            pltpu.SemaphoreType.DMA((8,)),
        ],
        compiler_params=pltpu.CompilerParams(
            vmem_limit_bytes=100 * 1024 * 1024, disable_semaphore_checks=True),
        interpret=interpret,
        name="hedgehog",
    )(x.reshape(S, D), wqkv, w_phi.reshape(H * DH, DH), wo)
    return out.reshape(1, S, D)


@jax.jit
def pallas_standalone__linear_kernel_hedgehog__prompt_kernel(
    x: jax.Array,
    wqkv: jax.Array,
    w_phi: jax.Array,
    wo: jax.Array,
):
    return _run(x, wqkv, w_phi, wo)
```

```python
import jax
import jax.numpy as jnp
from jax import lax
import jax.experimental.pallas as pl
import jax.experimental.pallas.tpu as pltpu

S, D, H, DH = 2048, 1024, 32, 32
TS = 256
T = S // TS
U2 = 3
RC = 32
LOG2E = 1.4426950408889634
NT = (((1,), (1,)), ((), ()))
NN = (((1,), (0,)), ((), ()))
TN = (((0,), (0,)), ((), ()))
f32, bf16 = jnp.float32, jnp.bfloat16


def _recip(x):
    r = pl.reciprocal(x, approx=True)
    return r * (2.0 - x * r)


def _allred(x, op):
    y = x[0:8]
    for i in range(1, x.shape[0] // 8):
        y = op(y, x[8 * i:8 * i + 8])
    y = op(y, pltpu.roll(y, 4, 0))
    return op(y, pltpu.roll(y, 2, 0))


def _pair_feat(p2):
    n = p2.shape[1]
    mx = _allred(p2, jnp.maximum)
    mn = _allred(p2, jnp.minimum)
    p3 = p2.reshape(8, 8, n)
    ep = jnp.exp2(p3 - mx[None]).reshape(64, n)
    en = jnp.exp2(mn[None] - p3).reshape(64, n)
    rp = _recip(_allred(ep, jnp.add))
    rn = _recip(_allred(en, jnp.add))
    a = (ep.reshape(8, 8, n) * rp[None]).reshape(64, n)
    b = (en.reshape(8, 8, n) * rn[None]).reshape(64, n)
    return jnp.concatenate([a, b], axis=0)


def _kernel(x_hbm, wqkv_hbm, wphi_hbm, wo_hbm, out_hbm,
            x_v, wq_v, wk_v, wv_v, wphi_v, wo_v, wkT, wqT, wvT, bd_v, kv_acc, kvb, zacc,
            car0, car7, cph7, carv, caro, acc, out_v, bdtmp, xu_v, sem):
    def cp_phi(a, b, s):
        rows = pl.ds(a * 128, (b - a) * 128)
        return pltpu.make_async_copy(wphi_hbm.at[rows, :], wphi_v.at[rows, :], sem.at[s])

    def cp_q(G, s):
        return pltpu.make_async_copy(wqkv_hbm.at[:, pl.ds(G * 128, 128)], wq_v.at[G], sem.at[s])

    def cp_k(G, s):
        return pltpu.make_async_copy(wqkv_hbm.at[:, pl.ds(D + G * 128, 128)], wk_v.at[G], sem.at[s])

    def cp_v(G, s):
        return pltpu.make_async_copy(wqkv_hbm.at[:, pl.ds(2 * D + G * 128, 128)], wv_v.at[G], sem.at[s])

    def cp_x(t, s):
        return pltpu.make_async_copy(x_hbm.at[pl.ds((t % T) * TS, TS), :], x_v.at[t], sem.at[s])

    def cp_x_dyn(t, s):
        r0 = pl.multiple_of(jnp.where(t >= T, 0, t) * TS, TS)
        return pltpu.make_async_copy(x_hbm.at[pl.ds(r0, TS), :], x_v.at[t], sem.at[s])

    def cp_q_dyn(G, s):
        cols = pl.ds(pl.multiple_of(G * 128, 128), 128)
        return pltpu.make_async_copy(wqkv_hbm.at[:, cols], wq_v.at[G], sem.at[s])

    cp_wo = pltpu.make_async_copy(wo_hbm, wo_v, sem.at[7])

    groups = [['p0', 'k0'], ['x0', 'k1'], ['p1', 'v0', 'k2'], ['p2', 'v1', 'k3'],
              ['v2', 'k4', 'v3', 'k5'], ['v4', 'k6', 'v5', 'k7', 'v6'], ['v7', 'x1', 'q0']]
    dmas = {}
    for s, grp in enumerate(groups):
        for n in grp:
            kind, i = n[0], int(n[1:])
            if kind == 'p':
                a, b = [(0, 2), (2, 4), (4, 8)][i]
                dmas[n] = lambda a=a, b=b, s=s: cp_phi(a, b, s)
            else:
                fn = {'q': cp_q, 'k': cp_k, 'v': cp_v, 'x': cp_x}[kind]
                dmas[n] = lambda fn=fn, i=i, s=s: fn(i, s)
    order = [n for grp in groups for n in grp]
    for i in range(7):
        dmas[f"x{i + 2}"] = lambda i=i: cp_x(i + 2, i)
        dmas[f"q{i + 1}"] = lambda i=i: cp_q(i + 1, i)
        order += [f"x{i + 2}", f"q{i + 1}"]
    dmas["o"] = lambda: cp_wo
    order += ["o"]
    pos = [0]

    def issue_to(name):
        last = len(order) - 1 if name is None else order.index(name)
        while pos[0] <= last:
            dmas[order[pos[0]]]().start()
            pos[0] += 1

    def wait(k):
        for n in groups[k]:
            assert order.index(n) < pos[0], n
            dmas[n]().wait()

    lane_head = lax.broadcasted_iota(jnp.int32, (32, 128), 1) // 32

    def BD(G):
        tm = wphi_v[G * 128:(G + 1) * 128, :].astype(f32).T
        for hh in range(4):
            rows = pl.ds(64 * (hh // 2) + hh % 2, 32, stride=2)
            bdtmp[G, rows, :] = jnp.where(lane_head == hh, tm, 0.0)
        bd_v[G] = bdtmp[G].astype(bf16)

    def fold(G, w_ref):
        w = lax.dot_general(bd_v[G], w_ref[G], NT, preferred_element_type=f32)
        return (w * LOG2E).astype(bf16)

    def Fk(G):
        wkT[G] = fold(G, wk_v)

    def Tv(G):
        wvT[G] = wv_v[G].T

    def xconv(t):
        xu_v[t] = pltpu.bitcast(x_v[t], jnp.uint32)

    def proj(w_ref, wi, t):
        return lax.dot_general(w_ref[wi], pltpu.bitcast(xu_v[t], bf16), NT, preferred_element_type=f32)

    def projv(G, t):
        return proj(wvT, G, t).astype(bf16)

    def SMk(p, G):
        out = []
        for j in range(2):
            ph = _pair_feat(p[64 * j:64 * j + 64])
            zacc[2 * G + j] += ph[:, 0:128] + ph[:, 128:256]
            out.append(ph.astype(bf16))
        return tuple(out)

    def den_r(ph, g):
        zb = zacc[g]
        cols = [_allred(ph[:, 128 * l:128 * l + 128] * zb, jnp.add) for l in range(TS // 128)]
        r = _recip(jnp.concatenate(cols, axis=1) + 1e-6)
        rs = pltpu.roll(r, 1, 0)
        even = (lax.broadcasted_iota(jnp.int32, (8, TS), 0) % 2) == 0
        return [jnp.where(even, r, rs), jnp.where(even, rs, r)]

    def SMq(p, G):
        out, rr = [], []
        for j in range(2):
            ph = _pair_feat(p[64 * j:64 * j + 64])
            rr.append(den_r(ph, 2 * G + j))
            out.append(ph.astype(bf16))
        return tuple(out), tuple(rr)

    def KV(phi, v, G, first):
        for j in range(2):
            g = 2 * G + j
            d = lax.dot_general(v[64 * j:64 * j + 64], phi[j], NT, preferred_element_type=f32)
            if not first:
                d = d + kv_acc[g]
            kv_acc[g] = d

    pk, ph, pv = {}, {}, {}
    issue_to('p1')
    zacc[...] = jnp.zeros(zacc.shape, f32)
    kv_acc[14] = jnp.zeros((64, 128), f32)
    kv_acc[15] = jnp.zeros((64, 128), f32)

    wait(0); issue_to('k2')
    BD(0); Fk(0); BD(1)

    wait(1); issue_to('k3')
    xconv(0)
    pk[0] = proj(wkT, 0, 0); Fk(1)

    wait(2); issue_to('k5')
    BD(2); Tv(0); BD(3)
    pk[1] = proj(wkT, 1, 0)
    ph[0] = SMk(pk.pop(0), 0)
    Fk(2)
    pv[0] = projv(0, 0)

    wait(3); issue_to('v6')
    Tv(1)
    pk[2] = proj(wkT, 2, 0)
    ph[1] = SMk(pk.pop(1), 1)
    for G in range(4, 8):
        BD(G)
    Fk(3)
    KV(ph.pop(0), pv.pop(0), 0, True)
    pv[1] = projv(1, 0)

    wait(4); issue_to('q0')
    Tv(2); Tv(3)
    pk[3] = proj(wkT, 3, 0)
    ph[2] = SMk(pk.pop(2), 2)
    Fk(4)
    KV(ph.pop(1), pv.pop(1), 1, True)
    pv[2] = projv(2, 0)
    pk[4] = proj(wkT, 4, 0)
    ph[3] = SMk(pk.pop(3), 3)
    Fk(5)
    KV(ph.pop(2), pv.pop(2), 2, True)
    pv[3] = projv(3, 0)

    wait(5); issue_to('q1')
    Tv(4); Tv(5); Tv(6)
    pk[5] = proj(wkT, 5, 0)
    ph[4] = SMk(pk.pop(4), 4)
    Fk(6)
    Fk(7)
    KV(ph.pop(3), pv.pop(3), 3, True)
    pv[4] = projv(4, 0)
    pk[6] = proj(wkT, 6, 0)
    ph[5] = SMk(pk.pop(5), 5)
    pv[5] = projv(5, 0)
    KV(ph.pop(4), pv.pop(4), 4, True)
    car7[...] = proj(wkT, 7, 0)
    ph[6] = SMk(pk.pop(6), 6)
    pv[6] = projv(6, 0)
    KV(ph.pop(5), pv.pop(5), 5, True)

    wait(6); issue_to(None)
    Tv(7)
    xconv(1)
    car0[...] = proj(wkT, 0, 1)
    q7 = SMk(car7[...], 7)
    cph7[0] = q7[0]
    cph7[1] = q7[1]
    wkT[8] = fold(0, wq_v)
    KV(ph.pop(6), pv.pop(6), 6, True)
    carv[...] = projv(7, 0)

    def phase1(i, carry):
        t = 1 + i
        cp_x_dyn(t + 1, i).wait()
        cp_q_dyn(t, i).wait()
        pk_ = car0[...]
        ph_ = {-1: (cph7[0], cph7[1])}
        pv_ = {-1: carv[...]}
        xconv(t + 1)
        for G in range(8):
            if G < 7:
                npk = proj(wkT, G + 1, t)
            else:
                npk = proj(wkT, jnp.where(t + 1 >= T, 8, 0), t + 1)
                car0[...] = npk
            pv_[G] = projv(G, t)
            if G == 7:
                carv[...] = pv_[G]
            KV(ph_.pop(G - 1), pv_.pop(G - 1), 7 if G == 0 else G - 1, False)
            ph_[G] = SMk(pk_, G)
            if G == 7:
                cph7[0] = ph_[G][0]
                cph7[1] = ph_[G][1]
            pk_ = npk
            if G == 3:
                wqT[i + 1] = fold(i + 1, wq_v)
        return carry

    lax.fori_loop(0, T - 1, phase1, 0)

    def N2(phi, rr, G):
        os_ = []
        for j in range(2):
            nd = lax.dot_general(kvb[2 * G + j], phi[j], NN, preferred_element_type=f32)
            os_ += [(nd[32 * e:32 * e + 32].reshape(4, 8, TS) * rr[j][e][None]).reshape(32, TS)
                    for e in range(2)]
        return jnp.concatenate(os_, axis=0).astype(bf16)

    def cp_out(t):
        return pltpu.make_async_copy(out_v.at[t], out_hbm.at[pl.ds(t * TS, TS), :], sem.at[0])

    def cp_out_chunk(t, m, n):
        return pltpu.make_async_copy(
            out_v.at[t, pl.ds(m * RC, RC), pl.ds(n * 512, 512)],
            out_hbm.at[pl.ds(t * TS + m * RC, RC), pl.ds(n * 512, 512)], sem.at[0])

    def OP(oT, t, G):
        res = lax.dot_general(oT, wo_v[G * 128:(G + 1) * 128, :], TN, preferred_element_type=f32)
        if G == 0:
            acc[...] = res
        elif G < 7:
            acc[...] += res
        else:
            out_v[t] = (acc[...] + res).astype(bf16)
            cp_out(t).start()

    def Q(G, t):
        return proj(wkT, 8, t) if G == 0 else proj(wqT, G, t)

    r = lax.broadcasted_iota(jnp.int32, (64, 128), 0)
    c = lax.broadcasted_iota(jnp.int32, (64, 128), 1)
    mask = (r // 32) == (c % 2)
    cp_wo.wait()
    for g in range(14):
        zacc[g] = jnp.broadcast_to(jnp.sum(zacc[g], axis=1, keepdims=True), (128, 128))
    for g in range(14):
        kvb[g] = jnp.where(mask, kv_acc[g], 0.0).astype(bf16)
    npq = Q(1, 0)
    phi, rr = SMq(car0[...], 0)
    ph7 = (cph7[0], cph7[1])
    oT = None
    for G in range(8):
        pq = npq
        if G == 1:
            for j in range(2):
                d = lax.dot_general(carv[64 * j:64 * j + 64], ph7[j], NT,
                                    preferred_element_type=f32) + kv_acc[14 + j]
                kvb[14 + j] = jnp.where(mask, d, 0.0).astype(bf16)
                zacc[14 + j] = jnp.broadcast_to(
                    jnp.sum(zacc[14 + j], axis=1, keepdims=True), (128, 128))
        if G < 6:
            npq = Q(G + 2, 0)
        elif G == 6:
            car0[...] = Q(0, 1)
        noT = N2(phi, rr, G)
        if G < 7:
            phi, rr = SMq(pq, G + 1)
        else:
            caro[...] = noT
        if G > 0:
            OP(oT, 0, G - 1)
        oT = noT

    def p2_tile(t, pq0, oT, store, final=False):
        npq = Q(1, t)
        phi, rr = SMq(pq0, 0)
        OP(oT, t - 1, 7)
        oT = N2(phi, rr, 0)
        phi, rr = SMq(npq, 1)
        nq0 = None
        for G in range(1, 8):
            if G < 7:
                pq = Q(G + 1, t)
            elif not final:
                nq0 = Q(0, t + 1)
                if store:
                    car0[...] = nq0
            noT = N2(phi, rr, G)
            if G < 7:
                phi, rr = SMq(pq, G + 1)
            elif store:
                caro[...] = noT
            OP(oT, t, G - 1)
            oT = noT
        return nq0, oT

    def phase2(i, carry):
        t = 1 + U2 * i
        pq0 = car0[...]
        oT = caro[...]
        for u in range(U2):
            pq0, oT = p2_tile(t + u, pq0, oT, u == U2 - 1)
        return carry

    lax.fori_loop(0, (T - 2) // U2, phase2, 0)

    t = T - 1
    npq = Q(1, t)
    phi, rr = SMq(car0[...], 0)
    OP(caro[...], t - 1, 7)
    oTs = {0: N2(phi, rr, 0)}
    phi, rr = SMq(npq, 1)
    for G in range(1, 8):
        if G < 7:
            pq = Q(G + 1, t)
        oTs[G] = N2(phi, rr, G)
        if G < 7:
            phi, rr = SMq(pq, G + 1)
        if G >= 2:
            OP(oTs.pop(G - 2), t, G - 2)
    o = jnp.concatenate([oTs.pop(6), oTs.pop(7)], axis=0).T
    for n in range(2):
        for m in range(TS // RC):
            rows, cols = slice(m * RC, (m + 1) * RC), slice(n * 512, (n + 1) * 512)
            res = jnp.dot(o[rows], wo_v[6 * 128:8 * 128, cols], preferred_element_type=f32)
            out_v[t, rows, cols] = (acc[rows, cols] + res).astype(bf16)
            cp_out_chunk(t, m, n).start()
    for tt in range(T - 1):
        cp_out(tt).wait()
    for n in range(2):
        for m in range(TS // RC):
            cp_out_chunk(t, m, n).wait()


def _run(x, wqkv, w_phi, wo, interpret=False):
    any_spec = pl.BlockSpec(memory_space=pl.ANY)
    out = pl.pallas_call(
        _kernel,
        out_shape=jax.ShapeDtypeStruct((S, D), bf16),
        in_specs=[any_spec] * 4,
        out_specs=any_spec,
        scratch_shapes=[
            pltpu.VMEM((T + 1, TS, D), bf16),
            pltpu.VMEM((8, D, 128), bf16),
            pltpu.VMEM((8, D, 128), bf16),
            pltpu.VMEM((8, D, 128), bf16),
            pltpu.VMEM((H * DH, DH), bf16),
            pltpu.VMEM((D, D), bf16),
            pltpu.VMEM((9, 128, D), bf16),
            pltpu.VMEM((8, 128, D), bf16),
            pltpu.VMEM((8, 128, D), bf16),
            pltpu.VMEM((8, 128, 128), bf16),
            pltpu.VMEM((16, 64, 128), f32),
            pltpu.VMEM((16, 64, 128), bf16),
            pltpu.VMEM((16, 128, 128), f32),
            pltpu.VMEM((128, TS), f32),
            pltpu.VMEM((128, TS), f32),
            pltpu.VMEM((2, 128, TS), bf16),
            pltpu.VMEM((128, TS), bf16),
            pltpu.VMEM((128, TS), bf16),
            pltpu.VMEM((TS, D), f32),
            pltpu.VMEM((T, TS, D), bf16),
            pltpu.VMEM((8, 128, 128), f32),
            pltpu.VMEM((T + 1, TS // 2, D), jnp.uint32),
            pltpu.SemaphoreType.DMA((8,)),
        ],
        compiler_params=pltpu.CompilerParams(
            vmem_limit_bytes=100 * 1024 * 1024, disable_semaphore_checks=True),
        interpret=interpret,
        name="hedgehog",
    )(x.reshape(S, D), wqkv, w_phi.reshape(H * DH, DH), wo)
    return out.reshape(1, S, D)


@jax.jit
def pallas_standalone__linear_kernel_hedgehog__prompt_kernel(
    x: jax.Array,
    wqkv: jax.Array,
    w_phi: jax.Array,
    wo: jax.Array,
):
    return _run(x, wqkv, w_phi, wo)
```
